```python
import jax
import jax.numpy as jnp

def _softmax(x, axis=-1):
    return jax.nn.softmax(x, axis=axis)

def _gelu(x):
    return jax.nn.gelu(x, approximate=True)

def _silu(x):
    return jax.nn.silu(x)

def _sigmoid(x):
    return jax.nn.sigmoid(x)

def _layernorm(x, axis=-1, eps=1e-05):
    m = jnp.mean(x, axis=axis, keepdims=True)
    v = jnp.var(x, axis=axis, keepdims=True)
    return (x - m) / jnp.sqrt(v + eps)

def _scatter_add(tgt, idx, src, axis=0):
    return tgt.at[idx].add(src)

def _segment_sum(src, seg, n):
    return jax.ops.segment_sum(src, seg, n)

class _Rng:

    def __init__(self, key):
        self._k = key

    def _next(self):
        self._k, sub = jax.random.split(self._k)
        return sub

    def normal(self, shape):
        return jax.random.normal(self._next(), shape, dtype=jnp.bfloat16)

    def randint(self, lo, hi, shape):
        return jax.random.randint(self._next(), shape, lo, hi, dtype=jnp.int32)

    def uniform(self, shape, lo=0.0, hi=1.0):
        return jax.random.uniform(self._next(), shape, jnp.bfloat16, lo, hi)

    def permutation(self, n):
        return jax.random.permutation(self._next(), n)
kernel_name = 'adaLN_cond__ssm_conv_h3__glu_gated_bilinear__prompt'

def setup_inputs():
    _rng = _Rng(jax.random.key(int.from_bytes(__import__("os").urandom(4), "little")))
    _w = lambda a: (lambda t: t.astype(jnp.bfloat16) if jnp.issubdtype(t.dtype, jnp.floating) else t)(jnp.asarray(a))

    def _A_setup():
        B, S, D = (1, 2048, 640)
        ks = 4
        return {'q': _w((lambda *s: _rng.normal(s) * 0.05)(B, S, D)), 'k': _w((lambda *s: _rng.normal(s) * 0.05)(B, S, D)), 'v': _w((lambda *s: _rng.normal(s) * 0.05)(B, S, D)), 'shift_k': _w((lambda *s: _rng.normal(s) * 0.05)(D, ks) * 0.5), 'ssm_k': _w((lambda *s: _rng.normal(s) * 0.05)(D, S) * (1.0 / S ** 0.5)), 'ssm_D': _w((lambda *s: _rng.normal(s) * 0.05)(D))}
    _A_in = _A_setup()

    def _B_setup():
        B, S, D, F = (1, 2048, 640, 1536)
        return {'x': _w((lambda *s: _rng.normal(s) * 0.05)(B, S, D)), 'w_gate': _w((lambda *s: _rng.normal(s) * 0.05)(D, F) * D ** (-0.5)), 'w_up': _w((lambda *s: _rng.normal(s) * 0.05)(D, F) * D ** (-0.5)), 'w_down': _w((lambda *s: _rng.normal(s) * 0.05)(F, D) * F ** (-0.5))}
    _B_in = _B_setup()
    return {'A_q': _A_in['q'], 'A_k': _A_in['k'], 'A_v': _A_in['v'], 'A_shift_k': _A_in['shift_k'], 'A_ssm_k': _A_in['ssm_k'], 'A_ssm_D': _A_in['ssm_D'], 'B_x': _B_in['x'], 'B_w_gate': _B_in['w_gate'], 'B_w_up': _B_in['w_up'], 'B_w_down': _B_in['w_down'], 'c': _w((lambda *s: _rng.normal(s) * 0.05)(1, 640)), 'w_mod': _w((lambda *s: _rng.normal(s) * 0.05)(640, 6 * 640) * 640 ** (-0.5))}

def reference(A_q, A_k, A_v, A_shift_k, A_ssm_k, A_ssm_D, B_x, B_w_gate, B_w_up, B_w_down, c, w_mod):

    def _A_ref(q, k, v, shift_k, ssm_k, ssm_D):
        B, S, D = q.shape
        ks = shift_k.shape[-1]
        k_pad = jnp.pad(k, ((0, 0), (ks - 1, 0), (0, 0)))
        k_shift = jnp.zeros_like(k)
        for t in range(ks):
            k_shift = k_shift + k_pad[:, t:t + S, :] * shift_k[:, ks - 1 - t][None, None, :]
        kv = k_shift * v
        L = 2 * S
        kv_pad = jnp.pad(kv, ((0, 0), (0, S), (0, 0)))
        kf_pad = jnp.pad(ssm_k, ((0, 0), (0, S)))
        kv_f = (lambda x, axes=(-2, -1): jnp.fft.rfft2(x.astype(jnp.float32), axes=axes))(kv_pad[:, None, :, :], axes=(1, 2))
        kf_f = (lambda x, axes=(-2, -1): jnp.fft.rfft2(x.astype(jnp.float32), axes=axes))(kf_pad[:, None, :], axes=(1, 2))
        kf_f = (lambda x, *d: x.transpose(*d))(kf_f, 1, 2, 0)
        y_f = kv_f * kf_f[None, :, :, :]
        y = (lambda x, s, axes=(-2, -1): jnp.fft.irfft2(x, s=s, axes=axes).astype(jnp.bfloat16))(y_f, (1, L), axes=(1, 2))[:, 0, :S, :]
        y = y + kv * ssm_D[None, None, :]
        return q * y

    def _B_ref(x, w_gate, w_up, w_down):
        g = jnp.einsum('bsd,df->bsf', x, w_gate)
        u = jnp.einsum('bsd,df->bsf', x, w_up)
        h = g * u
        return jnp.einsum('bsf,fd->bsd', h, w_down)
    x = A_q
    mod = (_silu(c) @ w_mod).reshape(c.shape[0], 6, 1, -1)
    sa, ca, ga, sb, cb, gb = (mod[:, 0].copy(), mod[:, 1].copy(), mod[:, 2].copy(), mod[:, 3].copy(), mod[:, 4].copy(), mod[:, 5].copy())
    h = _layernorm(x, axis=-1) * (1 + ca) + sa
    x = x + ga * _A_ref(h, A_k, A_v, A_shift_k, A_ssm_k, A_ssm_D)
    h = _layernorm(x, axis=-1) * (1 + cb) + sb
    x = x + gb * _B_ref(h, B_w_gate, B_w_up, B_w_down)
    return x
```

```python
import functools, itertools
import numpy as np
import jax
import jax.numpy as jnp
from jax.experimental import pallas as pl
from jax.experimental.pallas import tpu as pltpu

S, D, F = 2048, 640, 1536
C = 128
NCH = S // C
CPG = 2
M = C * CPG
NG = NCH // CPG
NF = F // 128
ND = D // 128
bf16 = jnp.bfloat16
f32 = jnp.float32
u32 = jnp.uint32
FLAGS = {}
OPT = dict(wm_first=20, wf=2, wbatch={2:(1,), 4:(2,3), 8:(4,5), 12:(6,7)}, tpro=tuple(range(8)), tplace={}, budget=(15, 6) + (20,)*6, post_chains=4, s1_chains=4, kv_chains=2, kv_chains_ss=1,
           mac0_chains=2, waitall_slot=2, stop_after=8, only_T=False, parts=('kv','x','k'), tord=2, horner=True)

OPT.update(dict(budget=(15,0,21,21,21,21,21,21)))

def _dft_consts():
    f = np.arange(128)
    perm = np.concatenate([f[0::2], f[1::2]])
    theta = np.pi * (2 * perm + 1) / 256.0
    n = np.arange(128)
    ang = theta[:, None] * n[None, :]
    Fm = np.concatenate([np.cos(ang), -np.sin(ang)], axis=0)
    Gm = Fm.T / 128.0
    return Fm, Gm

def dot(a, b):
    return jnp.dot(a, b, preferred_element_type=f32)

def dot_nt(a, b):
    return jax.lax.dot_general(a, b, (((1,), (1,)), ((), ())), preferred_element_type=f32)

def unpack(x):
    return pltpu.bitcast(x, bf16)

class Chain:
    def __init__(self, mask_fn):
        self.prev = None
        self.mask_fn = mask_fn
    def link(self, v):
        if self.prev is None:
            return v
        return jnp.where(self.mask_fn(v.shape), self.prev, v)
    def set(self, v):
        self.prev = v

def mac_schedule():
    budget = OPT['budget']; tplace = OPT['tplace']
    avail_g = max(OPT['tpro'])
    done = [set() for _ in range(NCH)]
    sched = []
    for s in range(NG):
        m = min(CPG * (avail_g + 1) - 1, NCH - 1)
        segs_due, segs_extra = [], []
        n = 0
        for i in range(CPG*s, CPG*(s+1)):
            js = [j for j in range(i + 1) if j not in done[i]]
            assert all(j <= m and i - j <= m for j in js), (s, i, js, m)
            if js:
                segs_due.append((i, js, len(done[i]) == 0, True))
                done[i].update(js); n += len(js)
        i = CPG * (s + 1)
        while n < budget[s] and i < NCH:
            js = [j for j in range(i + 1) if j not in done[i] and j <= m and i - j <= m]
            js = js[:budget[s] - n]
            if js:
                segs_extra.append((i, js, len(done[i]) == 0, len(done[i]) + len(js) == i + 1))
                done[i].update(js); n += len(js)
            i += 1
        sched.append((segs_extra, segs_due))
        if s in tplace: avail_g = max(tplace[s])
    assert all(len(done[i]) == i + 1 for i in range(NCH))
    return sched

def dma_order_names():
    tp = list(OPT['tpro'])
    order = []
    for g in tp: order += ['k%d'%g, 'v%d'%g, 's%d'%(2*g), 's%d'%(2*g+1)]
    order += ['q0', 'q1'] + ['wm%d'%i for i in range(25)]
    for f in range(NF): order += ['wg%d'%f, 'wu%d'%f]
    order += ['wm%d'%i for i in range(25, 30)] + ['wd%d'%j for j in range(ND)]
    rest = [g for g in range(NG) if g not in tp]
    for g in range(2, NG):
        order += ['q%d'%g]
    for g in rest: order += ['k%d'%g, 'v%d'%g, 's%d'%(2*g), 's%d'%(2*g+1)]
    assert len(order) == len(set(order)) == 99, len(order)
    if OPT['only_T']: order = [n for n in order if n[0] in 'kvs']
    return order
DMA_NAMES = ['k%d'%g for g in range(NG)] + ['v%d'%g for g in range(NG)] + ['q%d'%g for g in range(NG)] + ['s%d'%c for c in range(NCH)] + ['wm%d'%i for i in range(30)] + ['wg%d'%f for f in range(NF)] + ['wu%d'%f for f in range(NF)] + ['wd%d'%j for j in range(ND)]
def dma_order():
    return [DMA_NAMES.index(x) for x in dma_order_names()]

def pull(gen, n=None):
    if gen is None: return
    if n is None:
        for _ in gen: pass
    else:
        for _ in itertools.islice(gen, n): pass

def kernel(q_h, k_h, v_h, ssm_h, wg_h, wu_h, wd_h, wm_h,
           sk_ref, dv_ref, c_ref, fm_ref, gm_ref,
           out_h,
           q_v, k_v, v_v, ssm_v, wg_v, wu_v, wd_v, wm_v,
           x_s, k_s, kraw_s, kv_s, y_s, yt_s, x2_s, h2_s, p_s, o_s, vec_s, dn_s, yacc_s, fg_s, sems, osems):
    cps = {}
    def mk(name, src, dst):
        cps[name] = pltpu.make_async_copy(src, dst, sems.at[DMA_NAMES.index(name)])
    for g in range(NG):
        rows = pl.ds(g*M, M)
        mk('k%d'%g, k_h.at[rows, :], k_v.at[rows, :]); mk('v%d'%g, v_h.at[rows, :], v_v.at[rows, :]); mk('q%d'%g, q_h.at[rows, :], q_v.at[rows, :])
    for c in range(NCH): mk('s%d'%c, ssm_h.at[:, pl.ds(c*C, C)], ssm_v.at[c])
    for i in range(30): mk('wm%d'%i, wm_h.at[:, pl.ds(i*128, 128)], wm_v.at[i])
    for f in range(NF):
        mk('wg%d'%f, wg_h.at[:, pl.ds(f*128, 128)], wg_v.at[f]); mk('wu%d'%f, wu_h.at[:, pl.ds(f*128, 128)], wu_v.at[f])
    for j in range(ND): mk('wd%d'%j, wd_h.at[:, pl.ds(j*128, 128)], wd_v.at[j])
    def cp_o(g): return pltpu.make_async_copy(o_s.at[pl.ds(g*M, M), :], out_h.at[pl.ds(g*M, M), :], osems.at[g])
    waited = set()
    def W(name):
        if name not in waited:
            waited.add(name); cps[name].wait()
    for name in dma_order_names(): cps[name].start()

    wg_u, wu_u, wd_u, ssm_u, wm_u = (r.bitcast(u32) for r in (wg_v, wu_v, wd_v, ssm_v, wm_v))
    kv_u, y_u, h2_u, p_u, fg_u = (r.bitcast(u32) for r in (kv_s, y_s, h2_s, p_s, fg_s))
    fg_s[0] = fm_ref[...]
    fg_s[1, 0:128] = gm_ref[:, 0:128]
    fg_s[1, 128:256] = gm_ref[:, 128:256]
    Fm = lambda: unpack(fg_u[0])
    Gm = lambda: jnp.concatenate([unpack(fg_u[1, 0:64]), unpack(fg_u[1, 64:128])], axis=1)
    V_W, V_D, V_A1G, V_SAG, V_A2, V_SB, V_GB = 0, 4, 5, 6, 7, 8, 9
    skT = sk_ref[...].astype(f32)
    for j in range(4):
        vec_s[V_W + j] = jnp.broadcast_to(skT[j:j+1, :], (8, D))
    vec_s[V_D] = jnp.broadcast_to(dv_ref[...].astype(f32).reshape(1, D), (8, D))
    mask8 = jnp.broadcast_to(skT[0:1, 0:128], (8, 128)) * 0.0 > 1.0
    def mask_fn(shape):
        if shape == (8, 128): return mask8
        return jnp.concatenate([mask8] * (shape[1] // 128), axis=1)

    def compute_mod(idxs):
        cc = c_ref[...].astype(f32)
        s = (cc * jax.nn.sigmoid(cc)).astype(bf16)
        s16 = jnp.broadcast_to(s, (16, D))
        mods = {}
        for i in idxs:
            parts = []
            for j in range(ND):
                W('wm%d'%(i*ND + j))
                parts.append(dot(s16, unpack(wm_u[i*ND + j]))[0:8, :])
            mods[i] = jnp.concatenate(parts, axis=1)
        if 0 in idxs:
            vec_s[V_A1G] = (1 + mods[1]) * mods[2]
            vec_s[V_SAG] = mods[0] * mods[2]
            vec_s[V_A2] = 1 + mods[4]
            vec_s[V_SB] = mods[3]
        if 5 in idxs:
            vec_s[V_GB] = mods[5]

    row8 = jax.lax.broadcasted_iota(jnp.int32, (8, 128), 0)
    rowlt = [row8 < j for j in range(4)]
    kv_last = {}
    def KV(c, chains):
        g = c // CPG
        W('k%d'%g); W('v%d'%g)
        r0 = c * C
        wv = lambda j, cs: vec_s[V_W + j, :, cs]
        def shift(prev, cur, j):
            pz = jnp.zeros((8, 128), f32) if prev is None else prev
            return jnp.where(rowlt[j], pltpu.roll(pz, j, 0), pltpu.roll(cur, j, 0))
        prev = [None] * ND
        prevb = [None] * ND
        if c > 0:
            pv = k_v[pl.ds(r0 - 16, 16), :].astype(f32)
            for cc in range(ND):
                cs = slice(cc*128, (cc+1)*128)
                prev[cc] = pv[8:16, cs]
                if OPT['horner']:
                    prevb[cc] = pv[8:16, cs] * wv(2, cs) + shift(pv[0:8, cs], pv[8:16, cs], 1) * wv(3, cs)
        np_ = 0
        for r in range(r0, r0 + C, 16):
            kvs = []
            k16 = k_v[pl.ds(r, 16), :].astype(f32)
            v16 = v_v[pl.ds(r, 16), :].astype(f32)
            for hh in (0, 8):
                outs = []
                for cc in range(ND):
                    cs = slice(cc*128, (cc+1)*128)
                    ch = chains[np_ % len(chains)]; np_ += 1
                    kc = ch.link(k16[hh:hh+8, cs])
                    if OPT['horner']:
                        s1 = shift(prev[cc], kc, 1)
                        a = kc * wv(0, cs) + s1 * wv(1, cs)
                        b = kc * wv(2, cs) + s1 * wv(3, cs)
                        ks = a + shift(prevb[cc], b, 2)
                        prevb[cc] = b
                    else:
                        ks = kc * wv(0, cs)
                        for j in (1, 2, 3):
                            ks = ks + shift(prev[cc], kc, j) * wv(j, cs)
                    kvc = ks * v16[hh:hh+8, cs]
                    ch.set(kvc)
                    outs.append(kvc)
                    prev[cc] = kc
                kvs.append(outs)
            for j in range(ND):
                kv_s[j, pl.ds(r, 16), :] = jnp.concatenate([kvs[0][j], kvs[1][j]], 0).astype(bf16)
            yield
        kv_last[c] = chains[(np_ - 1) % len(chains)].prev

    def XT(c):
        r0 = c * C
        kvb = jnp.concatenate([unpack(kv_u[j, pl.ds(r0 // 2, C // 2), :]) for j in range(ND)], axis=1)
        x_s[c] = dot(Fm(), kvb)

    def KT(c):
        W('s%d'%c)
        Kc = dot_nt(Fm(), unpack(ssm_u[c]))
        if c == 0:
            k_s[c] = Kc
        else:
            Kp = kraw_s[(c - 1) % 2]
            k_s[c, 0:64, :] = Kc[0:64] - Kp[128:192]
            k_s[c, 64:128, :] = Kc[64:128] + Kp[192:256]
            k_s[c, 128:192, :] = Kc[128:192] + Kp[0:64]
            k_s[c, 192:256, :] = Kc[192:256] - Kp[64:128]
        if c < NCH - 1:
            kraw_s[c % 2] = Kc

    def mac_chains(n): return [(Chain(mask_fn), Chain(mask_fn)) for _ in range(n)]
    def MACsegs(segs, chains):
        npos = 0
        for (i, js, first, last) in segs:
            for r0 in range(0, 128, 16):
                for c0 in range(0, D, 128):
                    res = []
                    for rr in (r0, r0 + 8):
                        chr_, chi_ = chains[npos % len(chains)]; npos += 1
                        ar = ai = None
                        if not first:
                            ar = chr_.link(yacc_s[i, rr:rr+8, c0:c0+128])
                            ai = chi_.link(yacc_s[i, 128+rr:128+rr+8, c0:c0+128])
                        for j in js:
                            d = i - j
                            xr = x_s[j, rr:rr+8, c0:c0+128]; xi = x_s[j, 128+rr:128+rr+8, c0:c0+128]
                            kr = k_s[d, rr:rr+8, c0:c0+128]; ki = k_s[d, 128+rr:128+rr+8, c0:c0+128]
                            if ar is None:
                                t = chr_.link(xr*kr); t2 = chi_.link(xr*ki)
                                ar = t - xi*ki
                                ai = t2 + xi*kr
                            else:
                                ar = ar + xr*kr
                                ai = ai + xr*ki
                                ar = ar - xi*ki
                                ai = ai + xi*kr
                        chr_.set(ar); chi_.set(ai)
                        res.append((ar, ai))
                        if not last:
                            yacc_s[i, rr:rr+8, c0:c0+128] = ar
                            yacc_s[i, 128+rr:128+rr+8, c0:c0+128] = ai
                    if last:
                        y_s[i, c0 // 128, r0: r0 + 16, :] = jnp.concatenate([res[0][0], res[1][0]], 0).astype(bf16)
                        y_s[i, c0 // 128, 128 + r0: 128 + r0 + 16, :] = jnp.concatenate([res[0][1], res[1][1]], 0).astype(bf16)
                    yield

    def ln_stats(x):
        m = jnp.mean(x, axis=-1, keepdims=True)
        d = x - m
        v = jnp.mean(d * d, axis=-1, keepdims=True)
        return d * jax.lax.rsqrt(v + 1e-5)

    def S1(g, chains):
        W('q%d'%g)
        n = 0
        for r in range(g*M, (g+1)*M, 16):
            q16 = q_v[pl.ds(r, 16), :].astype(f32)
            for hh in (0, 8):
                ch = chains[n % len(chains)]; n += 1
                q = ch.link(q16[hh:hh+8])
                dn = ln_stats(q)
                ch.set(dn)
                dn_s[pl.ds(r + hh, 8), :] = dn
            yield

    def INV(c):
        yb = jnp.concatenate([unpack(y_u[c, j]) for j in range(ND)], axis=1)
        yt_s[c % 2] = dot(Gm(), yb)

    def POST(g, chains):
        n = 0
        for r in range(g*M, (g+1)*M, 16):
            c = r // C; rl = r % C
            hs = []
            kvv = jnp.concatenate([unpack(kv_u[j, pl.ds(r // 2, 8), :]) for j in range(ND)], axis=1).astype(f32)
            q16 = q_v[pl.ds(r, 16), :].astype(f32)
            for hh in (0, 8):
                ch = chains[n % len(chains)]; n += 1
                q = q16[hh:hh+8]
                y = ch.link(yt_s[c % 2, rl+hh:rl+hh+8, :])
                y = y + kvv[hh:hh+8] * vec_s[V_D]
                hg = dn_s[pl.ds(r + hh, 8), :] * vec_s[V_A1G] + vec_s[V_SAG]
                x2 = q + hg * y
                x2_s[pl.ds(r + hh, 8), :] = x2
                h2 = ln_stats(x2) * vec_s[V_A2] + vec_s[V_SB]
                ch.set(h2)
                hs.append(h2)
            hp = jnp.concatenate(hs, 0).astype(bf16)
            for j in range(ND):
                h2_s[j, pl.ds(r, 16), :] = hp[:, j*128:(j+1)*128]
            yield

    def GU(g, f):
        h = jnp.concatenate([unpack(h2_u[j, pl.ds(g*M // 2, M // 2), :]) for j in range(ND)], axis=1)
        W('wg%d'%f); W('wu%d'%f)
        gg = dot(h, unpack(wg_u[f])); uu = dot(h, unpack(wu_u[f]))
        p_s[g % 2, f] = (gg * uu).astype(bf16)

    def DN(g, j):
        p = jnp.concatenate([unpack(p_u[g % 2, f]) for f in range(NF)], axis=1)
        W('wd%d'%j)
        o = dot(p, unpack(wd_u[j]))
        cs = slice(j*128, (j+1)*128)
        gb = jnp.concatenate([vec_s[V_GB][:, cs]] * (M // 8), axis=0)
        o_s[pl.ds(g*M, M), cs] = (x2_s[pl.ds(g*M, M), cs] + gb * o).astype(bf16)
        if j == ND - 1:
            cp_o(g).start()

    def chains_of(n): return [Chain(mask_fn) for _ in range(n)]
    sched = mac_schedule()
    npieces = lambda segs: len(segs) * 40

    kvc = chains_of(OPT['kv_chains'])
    pro_c = [c for g in OPT['tpro'] for c in range(g*CPG, (g+1)*CPG)]
    v = OPT['tord']
    if v == 1:
        for c in pro_c: pull(KV(c, kvc)); XT(c); KT(c)
    elif v == 2:
        def Wg(g):
            for nm in ('k%d'%g, 'v%d'%g, 's%d'%(2*g), 's%d'%(2*g+1)): W(nm)
        Wg(pro_c[0] // CPG)
        pull(KV(pro_c[0], kvc))
        for c in pro_c:
            if c + 1 in pro_c:
                for g in OPT['wbatch'].get(c + 1, ()): Wg(g)
                pull(KV(c + 1, kvc))
            XT(c); KT(c)
    elif v == 3:
        for c in pro_c: KT(c); pull(KV(c, kvc)); XT(c)
    elif v == 4:
        for c in pro_c: pull(KV(c, kvc))
        for c in pro_c: XT(c); KT(c)
    elif v == 5:
        pull(KV(pro_c[0], kvc))
        for c in pro_c:
            kvn = KV(c + 1, kvc) if c + 1 in pro_c else None
            pull(kvn, 4); XT(c); pull(kvn, 4); KT(c)

    if OPT['only_T']:
        acc = x_s[0]
        for c in range(1, NCH): acc = acc + x_s[c] + k_s[c]
        o_s[0:M, :] = acc.astype(bf16)
        cp_o(0).start(); cp_o(0).wait()
        for name in dma_order_names(): W(name)
        return
    ex, due = sched[0]
    mc0 = mac_chains(OPT['mac0_chains'])
    pull(MACsegs(due, mc0))
    INV(0); INV(1)
    W('q0'); W('q1')
    s1p = chains_of(8)
    pull(S1(0, s1p)); pull(S1(1, s1p))
    pull(MACsegs(ex, mc0))
    for i in range(OPT['wm_first']): W('wm%d'%i)
    compute_mod(range(5))
    pull(POST(0, chains_of(8)))
    mch = mac_chains(1)
    s1c = chains_of(OPT['s1_chains']); pc = chains_of(OPT['post_chains'])
    for s in range(1, NG + 1):
        if s > OPT['stop_after']: break
        g = s - 1
        if s == 2: W('q2')
        if s == 3:
            for name in dma_order_names(): W(name)
        mac = post = None
        if s < NG:
            ex, due = sched[s]
            mac = MACsegs(ex + due, mch); nm = npieces(ex + due)
        for f in range(NF):
            if s == 1 and f % OPT['wf'] == 0:
                for ff in range(f, f + OPT['wf']): W('wg%d'%ff); W('wu%d'%ff)
            GU(g, f)
            if mac is not None and s == 1: pull(mac, (nm * (f+1)) // NF - (nm * f) // NF)
        pull(mac)
        if s < NG:
            INV(2*s); INV(2*s + 1)
            if s > 1: pull(S1(s, s1c))
            post = POST(s, pc)
        if g == 0: compute_mod([5])
        for j in range(ND):
            DN(g, j)
            if post is not None and s == 1: pull(post, (16 * (j+1)) // ND - (16 * j) // ND)
        pull(post)
    for name in dma_order_names(): W(name)
    for g in range(min(NG, OPT['stop_after'])): cp_o(g).wait()

@jax.jit
def pallas_adaLN_cond__ssm_conv_h3__glu_gated_bilinear__prompt_kernel(A_q, A_k, A_v, A_shift_k, A_ssm_k, A_ssm_D, B_x, B_w_gate, B_w_up, B_w_down, c, w_mod):
    Fm, Gm = _dft_consts()
    Fm = jnp.asarray(Fm, dtype=bf16); Gm = jnp.asarray(Gm, dtype=bf16)
    any_spec = pl.BlockSpec(memory_space=pl.ANY)
    vm = pl.BlockSpec(memory_space=pltpu.VMEM)
    nsem = len(DMA_NAMES)
    out = pl.pallas_call(
        kernel,
        in_specs=[any_spec]*8 + [vm]*5,
        out_specs=any_spec,
        out_shape=jax.ShapeDtypeStruct((S, D), bf16),
        scratch_shapes=[
            pltpu.VMEM((S, D), bf16), pltpu.VMEM((S, D), bf16), pltpu.VMEM((S, D), bf16),
            pltpu.VMEM((NCH, D, C), bf16),
            pltpu.VMEM((NF, D, 128), bf16), pltpu.VMEM((NF, D, 128), bf16), pltpu.VMEM((ND, F, 128), bf16),
            pltpu.VMEM((30, D, 128), bf16),
            pltpu.VMEM((NCH, 256, D), f32), pltpu.VMEM((NCH, 256, D), f32), pltpu.VMEM((2, 256, D), f32),
            pltpu.VMEM((ND, S, 128), bf16), pltpu.VMEM((NCH, ND, 256, 128), bf16), pltpu.VMEM((2, C, D), f32),
            pltpu.VMEM((S, D), f32), pltpu.VMEM((ND, S, 128), bf16), pltpu.VMEM((2, NF, M, 128), bf16), pltpu.VMEM((S, D), bf16),
            pltpu.VMEM((10, 8, D), f32), pltpu.VMEM((S, D), f32), pltpu.VMEM((NCH, 256, D), f32),
            pltpu.VMEM((2, 256, 128), bf16),
            pltpu.SemaphoreType.DMA((nsem,)), pltpu.SemaphoreType.DMA((NG,)),
        ],
        compiler_params=pltpu.CompilerParams(vmem_limit_bytes=110*1024*1024, flags=FLAGS),
    )(A_q.reshape(S, D), A_k.reshape(S, D), A_v.reshape(S, D), A_ssm_k, B_w_gate, B_w_up, B_w_down, w_mod,
      A_shift_k.T, A_ssm_D, c, Fm, Gm)
    return out.reshape(1, S, D)
```

```python
import functools, itertools, contextlib
import numpy as np
import jax
import jax.numpy as jnp
from jax.experimental import pallas as pl
from jax.experimental.pallas import tpu as pltpu

S, D, F = 2048, 640, 1536
C = 128
NCH = S // C
CPG = 2
M = C * CPG
NG = NCH // CPG
NF = F // 128
ND = D // 128
bf16 = jnp.bfloat16
f32 = jnp.float32
u32 = jnp.uint32
FLAGS = {}
OPT = dict(t_in_w1=False, dma_b2=10, kv_in_w3=True, t_block=True, dma_batch=69, dma_rest_at=-1, scopes=False, blocks=False, s1_pos='w1', ipos=12, mac_anchor=True, s1_first=True, s1_link=True, post0_chains=16, cut=None, wm_first=0, wf=4, wbatch={2:(1,)}, tpro=(0,1), tplace={1:(2,),2:(3,),3:(4,),4:(5,),5:(6,),6:(7,)}, budget=(10,6,19,20,20,20,20,21), post_chains=3, s1_chains=16, kv_chains=2, kv_chains_ss=3,
           mac0_chains=2, waitall_slot=4, stop_after=8, only_T=False, parts=('kv','x','k'), tord=2, horner=True)

OPT.update(dict())

def _dft_consts():
    f = np.arange(128)
    perm = np.concatenate([f[0::2], f[1::2]])
    theta = np.pi * (2 * perm + 1) / 256.0
    n = np.arange(128)
    ang = theta[:, None] * n[None, :]
    Fm = np.concatenate([np.cos(ang), -np.sin(ang)], axis=0)
    Gm = Fm.T / 128.0
    return Fm, Gm

def dot(a, b):
    return jnp.dot(a, b, preferred_element_type=f32)

def dot_nt(a, b):
    return jax.lax.dot_general(a, b, (((1,), (1,)), ((), ())), preferred_element_type=f32)

def unpack(x):
    return pltpu.bitcast(x, bf16)

class Chain:
    def __init__(self, mask_fn):
        self.prev = None
        self.mask_fn = mask_fn
    def link(self, v):
        if self.prev is None:
            return v
        return jnp.where(self.mask_fn(v.shape), self.prev, v)
    def set(self, v):
        self.prev = v

def mac_schedule():
    budget = OPT['budget']; tplace = OPT['tplace']
    avail_g = max(OPT['tpro'])
    done = [set() for _ in range(NCH)]
    sched = []
    for s in range(NG):
        m = min(CPG * (avail_g + 1) - 1, NCH - 1)
        segs_due, segs_extra = [], []
        n = 0
        for i in range(CPG*s, CPG*(s+1)):
            js = [j for j in range(i + 1) if j not in done[i]]
            assert all(j <= m and i - j <= m for j in js), (s, i, js, m)
            if js:
                segs_due.append((i, js, len(done[i]) == 0, True))
                done[i].update(js); n += len(js)
        i = CPG * (s + 1)
        while n < budget[s] and i < NCH:
            js = [j for j in range(i + 1) if j not in done[i] and j <= m and i - j <= m]
            js = js[:budget[s] - n]
            if js:
                segs_extra.append((i, js, len(done[i]) == 0, len(done[i]) + len(js) == i + 1))
                done[i].update(js); n += len(js)
            i += 1
        sched.append((segs_extra, segs_due))
        if s in tplace: avail_g = max(tplace[s])
    assert all(len(done[i]) == i + 1 for i in range(NCH))
    return sched

def dma_order_names():
    tp = list(OPT['tpro'])
    order = []
    for g in tp: order += ['k%d'%g, 'v%d'%g, 's%d'%(2*g), 's%d'%(2*g+1)]
    order += ['q0', 'q1'] + ['wm%d'%i for i in range(25)]
    for f in range(NF): order += ['wg%d'%f, 'wu%d'%f]
    for j in range(ND): order += ['wd%d'%j, 'wm%d'%(25 + j)]
    rest = [g for g in range(NG) if g not in tp]
    for g in range(2, NG):
        if g in rest: order += ['k%d'%g, 'v%d'%g, 's%d'%(2*g), 's%d'%(2*g+1)]
        order += ['q%d'%g]
    assert len(order) == len(set(order)) == 99, len(order)
    if OPT['only_T']: order = [n for n in order if n[0] in 'kvs']
    cut = OPT['cut']
    if cut:
        drop = ['q%d'%g for g in range(2, NG)]
        if cut in ('mac0', 'post0', 'gu0'): drop += ['wd%d'%j for j in range(ND)]
        if cut in ('mac0', 'post0'): drop += ['wg%d'%f for f in range(NF)] + ['wu%d'%f for f in range(NF)]
        if cut == 'mac0': drop += ['wm%d'%i for i in range(30)]
        order = [n for n in order if n not in drop]
    return order
DMA_NAMES = ['k%d'%g for g in range(NG)] + ['v%d'%g for g in range(NG)] + ['q%d'%g for g in range(NG)] + ['s%d'%c for c in range(NCH)] + ['wm%d'%i for i in range(30)] + ['wg%d'%f for f in range(NF)] + ['wu%d'%f for f in range(NF)] + ['wd%d'%j for j in range(ND)]
def dma_order():
    return [DMA_NAMES.index(x) for x in dma_order_names()]

def pull(gen, n=None):
    if gen is None: return
    if n is None:
        for _ in gen: pass
    else:
        for _ in itertools.islice(gen, n): pass

def kernel(q_h, k_h, v_h, ssm_h, wg_h, wu_h, wd_h, wm_h,
           sk_ref, dv_ref, c_ref, fm_ref, gm_ref, z_ref,
           out_h,
           q_v, k_v, v_v, ssm_v, wg_v, wu_v, wd_v, wm_v,
           x_s, k_s, kraw_s, kv_s, y_s, yt_s, x2_s, h2_s, p_s, o_s, vec_s, dn_s, yacc_s, fg_s, sems, osems):
    cps = {}
    def mk(name, src, dst):
        cps[name] = pltpu.make_async_copy(src, dst, sems.at[DMA_NAMES.index(name)])
    for g in range(NG):
        rows = pl.ds(g*M, M)
        mk('k%d'%g, k_h.at[rows, :], k_v.at[rows, :]); mk('v%d'%g, v_h.at[rows, :], v_v.at[rows, :]); mk('q%d'%g, q_h.at[rows, :], q_v.at[rows, :])
    for c in range(NCH): mk('s%d'%c, ssm_h.at[:, pl.ds(c*C, C)], ssm_v.at[c])
    for i in range(30): mk('wm%d'%i, wm_h.at[:, pl.ds(i*128, 128)], wm_v.at[i])
    for f in range(NF):
        mk('wg%d'%f, wg_h.at[:, pl.ds(f*128, 128)], wg_v.at[f]); mk('wu%d'%f, wu_h.at[:, pl.ds(f*128, 128)], wu_v.at[f])
    for j in range(ND): mk('wd%d'%j, wd_h.at[:, pl.ds(j*128, 128)], wd_v.at[j])
    def cp_o(g): return pltpu.make_async_copy(o_s.at[pl.ds(g*M, M), :], out_h.at[pl.ds(g*M, M), :], osems.at[g])
    waited = set()
    def W(name):
        if name not in waited:
            waited.add(name); cps[name].wait()
    names = dma_order_names()
    nb1 = OPT['dma_batch']
    for name in names[:nb1]: cps[name].start()
    started = [nb1]
    def start_rest(n=None):
        n = len(names) - started[0] if n is None else min(n, len(names) - started[0])
        for name in names[started[0]:started[0] + n]: cps[name].start()
        started[0] += n

    wg_u, wu_u, wd_u, ssm_u, wm_u = (r.bitcast(u32) for r in (wg_v, wu_v, wd_v, ssm_v, wm_v))
    kv_u, y_u, h2_u, p_u, fg_u = (r.bitcast(u32) for r in (kv_s, y_s, h2_s, p_s, fg_s))
    fg_s[0] = fm_ref[...]
    fg_s[1, 0:128] = gm_ref[:, 0:128]
    fg_s[1, 128:256] = gm_ref[:, 128:256]
    Fm = lambda: unpack(fg_u[0])
    Gm = lambda: jnp.concatenate([unpack(fg_u[1, 0:64]), unpack(fg_u[1, 64:128])], axis=1)
    V_W, V_D, V_A1G, V_SAG, V_A2, V_SB, V_GB = 0, 4, 5, 6, 7, 8, 9
    skT = sk_ref[...].astype(f32)
    for j in range(4):
        vec_s[V_W + j] = jnp.broadcast_to(skT[j:j+1, :], (8, D))
    vec_s[V_D] = jnp.broadcast_to(dv_ref[...].astype(f32).reshape(1, D), (8, D))
    mask8 = jnp.broadcast_to(skT[0:1, 0:128], (8, 128)) * 0.0 > 1.0
    def mask_fn(shape):
        if shape == (8, 128): return mask8
        return jnp.concatenate([mask8] * (shape[1] // 128), axis=1)

    def silu_c():
        cc = c_ref[...].astype(f32)
        return jnp.broadcast_to((cc * jax.nn.sigmoid(cc)).astype(bf16), (16, D))
    def compute_mod(idxs):
        s16 = silu_c()
        mods = {}
        for i in idxs:
            parts = []
            for j in range(ND): W('wm%d'%(i*ND + j))
            for j in range(ND):
                W('wm%d'%(i*ND + j))
                parts.append(dot(s16, unpack(wm_u[i*ND + j]))[0:8, :])
            mods[i] = jnp.concatenate(parts, axis=1)
        if 0 in idxs:
            vec_s[V_A1G] = (1 + mods[1]) * mods[2]
            vec_s[V_SAG] = mods[0] * mods[2]
            vec_s[V_A2] = 1 + mods[4]
            vec_s[V_SB] = mods[3]
        if 5 in idxs:
            vec_s[V_GB] = mods[5]

    row8 = jax.lax.broadcasted_iota(jnp.int32, (8, 128), 0)
    rowlt = [row8 < j for j in range(4)]
    kv_last = {}
    def KV(c, chains):
        g = c // CPG
        W('k%d'%g); W('v%d'%g)
        r0 = c * C
        wv = lambda j, cs: vec_s[V_W + j, :, cs]
        def shift(prev, cur, j):
            pz = jnp.zeros((8, 128), f32) if prev is None else prev
            return jnp.where(rowlt[j], pltpu.roll(pz, j, 0), pltpu.roll(cur, j, 0))
        prev = [None] * ND
        prevb = [None] * ND
        if c > 0:
            pv = k_v[pl.ds(r0 - 16, 16), :].astype(f32)
            for cc in range(ND):
                cs = slice(cc*128, (cc+1)*128)
                prev[cc] = pv[8:16, cs]
                if OPT['horner']:
                    prevb[cc] = pv[8:16, cs] * wv(2, cs) + shift(pv[0:8, cs], pv[8:16, cs], 1) * wv(3, cs)
        np_ = 0
        for r in range(r0, r0 + C, 16):
            kvs = []
            k16 = k_v[pl.ds(r, 16), :].astype(f32)
            v16 = v_v[pl.ds(r, 16), :].astype(f32)
            for hh in (0, 8):
                outs = []
                for cc in range(ND):
                    cs = slice(cc*128, (cc+1)*128)
                    ch = chains[np_ % len(chains)]; np_ += 1
                    kc = ch.link(k16[hh:hh+8, cs])
                    if OPT['horner']:
                        s1 = shift(prev[cc], kc, 1)
                        a = kc * wv(0, cs) + s1 * wv(1, cs)
                        b = kc * wv(2, cs) + s1 * wv(3, cs)
                        ks = a + shift(prevb[cc], b, 2)
                        prevb[cc] = b
                    else:
                        ks = kc * wv(0, cs)
                        for j in (1, 2, 3):
                            ks = ks + shift(prev[cc], kc, j) * wv(j, cs)
                    kvc = ks * v16[hh:hh+8, cs]
                    ch.set(kvc)
                    outs.append(kvc)
                    prev[cc] = kc
                kvs.append(outs)
            for j in range(ND):
                kv_s[j, pl.ds(r, 16), :] = jnp.concatenate([kvs[0][j], kvs[1][j]], 0).astype(bf16)
            yield
        kv_last[c] = chains[(np_ - 1) % len(chains)].prev

    def XT(c):
        r0 = c * C
        kvb = jnp.concatenate([unpack(kv_u[j, pl.ds(r0 // 2, C // 2), :]) for j in range(ND)], axis=1)
        x_s[c] = dot(Fm(), kvb)

    def KT(c):
        W('s%d'%c)
        Kc = dot_nt(Fm(), unpack(ssm_u[c]))
        if c == 0:
            k_s[c] = Kc
        else:
            Kp = kraw_s[(c - 1) % 2]
            k_s[c, 0:64, :] = Kc[0:64] - Kp[128:192]
            k_s[c, 64:128, :] = Kc[64:128] + Kp[192:256]
            k_s[c, 128:192, :] = Kc[128:192] + Kp[0:64]
            k_s[c, 192:256, :] = Kc[192:256] - Kp[64:128]
        if c < NCH - 1:
            kraw_s[c % 2] = Kc

    def mac_chains(n): return [(Chain(mask_fn), Chain(mask_fn)) for _ in range(n)]
    def MACsegs(segs, chains):
        npos = 0
        for (i, js, first, last) in segs:
            for r0 in range(0, 128, 16):
                for c0 in range(0, D, 128):
                    res = []
                    for rr in (r0, r0 + 8):
                        chr_, chi_ = chains[npos % len(chains)]; npos += 1
                        ar = ai = None
                        if not first:
                            ar = chr_.link(yacc_s[i, rr:rr+8, c0:c0+128])
                            ai = chi_.link(yacc_s[i, 128+rr:128+rr+8, c0:c0+128])
                        for j in js:
                            d = i - j
                            xr = x_s[j, rr:rr+8, c0:c0+128]; xi = x_s[j, 128+rr:128+rr+8, c0:c0+128]
                            kr = k_s[d, rr:rr+8, c0:c0+128]; ki = k_s[d, 128+rr:128+rr+8, c0:c0+128]
                            if ar is None:
                                t = chr_.link(xr*kr); t2 = chi_.link(xr*ki)
                                ar = t - xi*ki
                                ai = t2 + xi*kr
                            else:
                                ar = ar + xr*kr
                                ai = ai + xr*ki
                                ar = ar - xi*ki
                                ai = ai + xi*kr
                        chr_.set(ar); chi_.set(ai)
                        res.append((ar, ai))
                        if not last:
                            yacc_s[i, rr:rr+8, c0:c0+128] = ar
                            yacc_s[i, 128+rr:128+rr+8, c0:c0+128] = ai
                    if last:
                        y_s[i, c0 // 128, r0: r0 + 16, :] = jnp.concatenate([res[0][0], res[1][0]], 0).astype(bf16)
                        y_s[i, c0 // 128, 128 + r0: 128 + r0 + 16, :] = jnp.concatenate([res[0][1], res[1][1]], 0).astype(bf16)
                    yield

    def ln_stats(x):
        m = jnp.mean(x, axis=-1, keepdims=True)
        d = x - m
        v = jnp.mean(d * d, axis=-1, keepdims=True)
        return d * jax.lax.rsqrt(v + 1e-5)

    def S1(g, chains):
        W('q%d'%g)
        n = 0
        for r in range(g*M, (g+1)*M, 16):
            q16 = q_v[pl.ds(r, 16), :].astype(f32)
            for hh in (0, 8):
                ch = chains[n % len(chains)]; n += 1
                q = ch.link(q16[hh:hh+8])
                dn = ln_stats(q)
                ch.set(dn)
                dn_s[pl.ds(r + hh, 8), :] = dn
            yield

    def anchored(w, anchors):
        if not anchors: return w
        w0 = w[0:8]
        for a in anchors:
            w0 = jnp.where(mask8, pltpu.bitcast(a, u32), w0)
        return jnp.concatenate([w0, w[8:]], axis=0)

    def INV(c, anchors=()):
        yb = jnp.concatenate([unpack(anchored(y_u[c, j], anchors if j == 0 else ())) for j in range(ND)], axis=1)
        yt_s[c % 2] = dot(Gm(), yb)

    def POST(g, chains):
        n = 0
        for r in range(g*M, (g+1)*M, 16):
            c = r // C; rl = r % C
            hs = []
            kvv = jnp.concatenate([unpack(kv_u[j, pl.ds(r // 2, 8), :]) for j in range(ND)], axis=1).astype(f32)
            q16 = q_v[pl.ds(r, 16), :].astype(f32)
            for hh in (0, 8):
                ch = chains[n % len(chains)]; n += 1
                q = q16[hh:hh+8]
                y = ch.link(yt_s[c % 2, rl+hh:rl+hh+8, :])
                y = y + kvv[hh:hh+8] * vec_s[V_D]
                hg = dn_s[pl.ds(r + hh, 8), :] * vec_s[V_A1G] + vec_s[V_SAG]
                x2 = q + hg * y
                x2_s[pl.ds(r + hh, 8), :] = x2
                h2 = ln_stats(x2) * vec_s[V_A2] + vec_s[V_SB]
                ch.set(h2)
                hs.append(h2)
            hp = jnp.concatenate(hs, 0).astype(bf16)
            for j in range(ND):
                h2_s[j, pl.ds(r, 16), :] = hp[:, j*128:(j+1)*128]
            yield

    def GU(g, f):
        h = jnp.concatenate([unpack(h2_u[j, pl.ds(g*M // 2, M // 2), :]) for j in range(ND)], axis=1)
        W('wg%d'%f); W('wu%d'%f)
        gg = dot(h, unpack(wg_u[f])); uu = dot(h, unpack(wu_u[f]))
        p_s[g % 2, f] = (gg * uu).astype(bf16)

    def DN(g, j):
        p = jnp.concatenate([unpack(p_u[g % 2, f]) for f in range(NF)], axis=1)
        W('wd%d'%j)
        o = dot(p, unpack(wd_u[j]))
        cs = slice(j*128, (j+1)*128)
        gb = jnp.concatenate([vec_s[V_GB][:, cs]] * (M // 8), axis=0)
        o_s[pl.ds(g*M, M), cs] = (x2_s[pl.ds(g*M, M), cs] + gb * o).astype(bf16)
        if j == ND - 1:
            cp_o(g).start()

    def chains_of(n): return [Chain(mask_fn) for _ in range(n)]
    sched = mac_schedule()
    npieces = lambda segs: len(segs) * 40

    sc = (lambda n: jax.named_scope(n)) if OPT['scopes'] else (lambda n: contextlib.nullcontext())
    kvc = chains_of(OPT['kv_chains'])
    pro_c = [c for g in OPT['tpro'] for c in range(g*CPG, (g+1)*CPG)]
    v = OPT['tord']
    if v == 1:
        for c in pro_c: pull(KV(c, kvc)); XT(c); KT(c)
    elif v == 2:
        def Wg(g):
            for nm in ('k%d'%g, 'v%d'%g, 's%d'%(2*g), 's%d'%(2*g+1)): W(nm)
        with sc('T'):
            Wg(pro_c[0] // CPG)
            pull(KV(pro_c[0], kvc))
            for c in pro_c:
                if c + 1 in pro_c:
                    for g in OPT['wbatch'].get(c + 1, ()): Wg(g)
                    pull(KV(c + 1, kvc))
                XT(c); KT(c)
                if c == OPT['dma_rest_at']: start_rest()
    elif v == 3:
        for c in pro_c: KT(c); pull(KV(c, kvc)); XT(c)
    elif v == 4:
        for c in pro_c: pull(KV(c, kvc))
        for c in pro_c: XT(c); KT(c)
    elif v == 5:
        pull(KV(pro_c[0], kvc))
        for c in pro_c:
            kvn = KV(c + 1, kvc) if c + 1 in pro_c else None
            pull(kvn, 4); XT(c); pull(kvn, 4); KT(c)

    if OPT['only_T']:
        acc = x_s[0]
        for c in range(1, NCH): acc = acc + x_s[c] + k_s[c]
        o_s[0:M, :] = acc.astype(bf16)
        cp_o(0).start(); cp_o(0).wait()
        for name in dma_order_names(): W(name)
        return
    ex, due = sched[0]
    mc0 = mac_chains(OPT['mac0_chains'])
    with sc('MAC0'):
        pull(MACsegs(due, mc0))
        INV(0); INV(1)
        W('q0'); W('q1')
        s1p = chains_of(8)
        pull(S1(0, s1p)); pull(S1(1, s1p))
        pull(MACsegs(ex, mc0))
    def finish(val):
        o_s[0:M, :] = val.astype(bf16)
        cp_o(0).start(); cp_o(0).wait()
        for name in dma_order_names(): W(name)
    if OPT['cut'] == 'mac0':
        finish(dn_s[0:M, :] + yacc_s[4, 0:M, :] + dn_s[M:2*M, :]); return
    with sc('WMWAIT'):
        for i in range(OPT['wm_first']): W('wm%d'%i)
    start_rest(OPT['dma_b2'])
    with sc('MOD'):
        compute_mod(range(5))
    with sc('POST0'):
        pull(POST(0, chains_of(OPT['post0_chains'])))
    if OPT['cut'] == 'post0':
        finish(jnp.concatenate([unpack(h2_u[j, 0:M//2, :]) for j in range(ND)], axis=1)); return
    ztrue = z_ref[0] == 0
    def block(fn, on):
        if on: pl.when(ztrue)(fn)
        else: fn()
    for s in range(1, NG + 1):
        if s > OPT['stop_after']: break
        g = s - 1
        if s == 2: start_rest()
        if 2 <= s < NG:
            W('q%d'%s)
            for tg in OPT['tplace'].get(s, ()): W('k%d'%tg); W('v%d'%tg)
        if s == OPT['waitall_slot']:
            for name in dma_order_names(): W(name)
        useblk = OPT['blocks'] and s >= 2
        def TT(s):
            kc = chains_of(OPT['kv_chains'])
            for tg in OPT['tplace'].get(s, ()):
                for nm_ in ('k%d'%tg, 'v%d'%tg, 's%d'%(2*tg), 's%d'%(2*tg+1)): W(nm_)
                c0 = tg * CPG
                if not (OPT['kv_in_w3'] and s > 1): pull(KV(c0, kc)); pull(KV(c0 + 1, kc))
                XT(c0); KT(c0); XT(c0 + 1); KT(c0 + 1)
        def W1(s=s, g=g):
            mch = mac_chains(1); s1c = chains_of(OPT['s1_chains'])
            mac = None
            if OPT['t_in_w1'] and s >= 2: TT(s - 1)
            if s < NG:
                ex, due = sched[s]
                if OPT['s1_pos'] == 'w1' and s > 1:
                    pull(S1(s, s1c))
                    if OPT['s1_link']:
                        lv = s1c[-1].prev[:, 0:128]
                        mch[0][0].set(lv); mch[0][1].set(lv)
                mac = MACsegs(ex + due, mch); nm = npieces(ex + due)
            for f in range(NF):
                if s == 1 and f % OPT['wf'] == 0:
                    for ff in range(f, f + OPT['wf']): W('wg%d'%ff); W('wu%d'%ff)
                GU(g, f)
                if mac is not None and s == 1: pull(mac, (nm * (f+1)) // NF - (nm * f) // NF)
            pull(mac)
        def W3(s=s, g=g):
            pc = chains_of(OPT['post_chains']); s1c = chains_of(OPT['s1_chains'])
            post = None
            if s < NG:
                INV(2*s); INV(2*s + 1)
                post = POST(s, pc)
            for j in range(ND):
                if s == 1:
                    W('wd%d'%j); W('wm%d'%(25 + j))
                    vec_s[V_GB, :, j*128:(j+1)*128] = dot(silu_c(), unpack(wm_u[25 + j]))[0:8, :]
                DN(g, j)
                if s == 1: pull(post, (16 * (j+1)) // ND - (16 * j) // ND)
            pull(post)
            if OPT['s1_pos'] == 'w3' and 1 <= s < NG - 1: pull(S1(s + 1, s1c))
            if OPT['kv_in_w3'] and s > 1:
                kc = chains_of(OPT['kv_chains_ss'])
                for tg in OPT['tplace'].get(s, ()):
                    W('k%d'%tg); W('v%d'%tg)
                    pull(KV(tg * CPG, kc)); pull(KV(tg * CPG + 1, kc))
            if not OPT['t_block'] and not OPT['t_in_w1']: TT(s)
        with sc('W1_%d'%s): block(W1, useblk)
        with sc('W3_%d'%s): block(W3, useblk)
        if OPT['t_block'] and not OPT['t_in_w1'] and s in OPT['tplace']:
            with sc('T_%d'%s): block(functools.partial(TT, s), True)
    for name in dma_order_names(): W(name)
    for g in range(min(NG, OPT['stop_after'])): cp_o(g).wait()

@jax.jit
def pallas_adaLN_cond__ssm_conv_h3__glu_gated_bilinear__prompt_kernel(A_q, A_k, A_v, A_shift_k, A_ssm_k, A_ssm_D, B_x, B_w_gate, B_w_up, B_w_down, c, w_mod):
    Fm, Gm = _dft_consts()
    Fm = jnp.asarray(Fm, dtype=bf16); Gm = jnp.asarray(Gm, dtype=bf16)
    any_spec = pl.BlockSpec(memory_space=pl.ANY)
    vm = pl.BlockSpec(memory_space=pltpu.VMEM)
    nsem = len(DMA_NAMES)
    out = pl.pallas_call(
        kernel,
        in_specs=[any_spec]*8 + [vm]*5 + [pl.BlockSpec(memory_space=pltpu.SMEM)],
        out_specs=any_spec,
        out_shape=jax.ShapeDtypeStruct((S, D), bf16),
        scratch_shapes=[
            pltpu.VMEM((S, D), bf16), pltpu.VMEM((S, D), bf16), pltpu.VMEM((S, D), bf16),
            pltpu.VMEM((NCH, D, C), bf16),
            pltpu.VMEM((NF, D, 128), bf16), pltpu.VMEM((NF, D, 128), bf16), pltpu.VMEM((ND, F, 128), bf16),
            pltpu.VMEM((30, D, 128), bf16),
            pltpu.VMEM((NCH, 256, D), f32), pltpu.VMEM((NCH, 256, D), f32), pltpu.VMEM((2, 256, D), f32),
            pltpu.VMEM((ND, S, 128), bf16), pltpu.VMEM((NCH, ND, 256, 128), bf16), pltpu.VMEM((2, C, D), f32),
            pltpu.VMEM((S, D), f32), pltpu.VMEM((ND, S, 128), bf16), pltpu.VMEM((2, NF, M, 128), bf16), pltpu.VMEM((S, D), bf16),
            pltpu.VMEM((10, 8, D), f32), pltpu.VMEM((S, D), f32), pltpu.VMEM((NCH, 256, D), f32),
            pltpu.VMEM((2, 256, 128), bf16),
            pltpu.SemaphoreType.DMA((nsem,)), pltpu.SemaphoreType.DMA((NG,)),
        ],
        compiler_params=pltpu.CompilerParams(vmem_limit_bytes=110*1024*1024, flags=FLAGS),
    )(A_q.reshape(S, D), A_k.reshape(S, D), A_v.reshape(S, D), A_ssm_k, B_w_gate, B_w_up, B_w_down, w_mod,
      A_shift_k.T, A_ssm_D, c, Fm, Gm, np.zeros((8,), np.int32))
    return out.reshape(1, S, D)
```

```python
import itertools

import numpy as np
import jax
import jax.numpy as jnp
from jax.experimental import pallas as pl
from jax.experimental.pallas import tpu as pltpu

S, D, F = 2048, 640, 1536
C = 128
NCH = S // C
CPG = 2
M = C * CPG
NG = NCH // CPG
NF = F // 128
ND = D // 128
bf16 = jnp.bfloat16
f32 = jnp.float32
u32 = jnp.uint32

T_PROLOGUE = (0, 1)
T_PLACE = {s: s + 1 for s in range(1, NG - 1)}
MAC_BUDGET = (10, 6, 19, 20, 20, 20, 20, 20)
FIRST_DMA_BATCH, SECOND_DMA_BATCH = 69, 10
GU_WAITS = {0: (0,), 1: (1,), 2: (2, 3), 4: (4, 5, 6, 7), 8: (8, 9, 10, 11)}


def _dft_consts():
    f = np.arange(128)
    perm = np.concatenate([f[0::2], f[1::2]])
    theta = np.pi * (2 * perm + 1) / 256.0
    ang = theta[:, None] * np.arange(128)[None, :]
    fm = np.concatenate([np.cos(ang), -np.sin(ang)], axis=0)
    gm = fm.T / 128.0
    return fm, gm


def _dot(a, b):
    return jnp.dot(a, b, preferred_element_type=f32)


def _dot_nt(a, b):
    return jax.lax.dot_general(a, b, (((1,), (1,)), ((), ())), preferred_element_type=f32)


def _unpack(x):
    return pltpu.bitcast(x, bf16)


class Chain:
    def __init__(self, mask_fn):
        self.prev = None
        self.mask_fn = mask_fn

    def link(self, v):
        if self.prev is None:
            return v
        return jnp.where(self.mask_fn(v.shape), self.prev, v)

    def set(self, v):
        self.prev = v


def _mac_schedule():
    avail_g = max(T_PROLOGUE)
    done = [set() for _ in range(NCH)]
    sched = []
    for s in range(NG):
        m = min(CPG * (avail_g + 1) - 1, NCH - 1)
        due, extra = [], []
        n = 0
        for i in range(CPG * s, CPG * (s + 1)):
            js = [j for j in range(i + 1) if j not in done[i]]
            assert all(j <= m and i - j <= m for j in js)
            if js:
                due.append((i, js, len(done[i]) == 0, True))
                done[i].update(js)
                n += len(js)
        i = CPG * (s + 1)
        while n < MAC_BUDGET[s] and i < NCH:
            js = [j for j in range(i + 1) if j not in done[i] and j <= m and i - j <= m]
            js = js[:MAC_BUDGET[s] - n]
            if js:
                extra.append((i, js, len(done[i]) == 0, len(done[i]) + len(js) == i + 1))
                done[i].update(js)
                n += len(js)
            i += 1
        sched.append((extra, due))
        if s in T_PLACE:
            avail_g = T_PLACE[s]
    assert all(len(done[i]) == i + 1 for i in range(NCH))
    return sched


def _group_names(g):
    return ['k%d' % g, 'v%d' % g] + ['s%d' % c for c in range(g * CPG, (g + 1) * CPG)]


DMA_NAMES = (['k%d' % g for g in range(NG)] + ['v%d' % g for g in range(NG)]
             + ['q%d' % g for g in range(NG)] + ['s%d' % c for c in range(NCH)]
             + ['wm%d' % i for i in range(6 * ND)] + ['wg%d' % f for f in range(NF)]
             + ['wu%d' % f for f in range(NF)] + ['wd%d' % j for j in range(ND)])


def _dma_order():
    order = []
    for g in T_PROLOGUE:
        order += _group_names(g)
    order += ['q0', 'q1'] + ['wm%d' % i for i in range(5 * ND)]
    for f in range(NF):
        order += ['wg%d' % f, 'wu%d' % f]
    for j in range(ND):
        order += ['wd%d' % j, 'wm%d' % (5 * ND + j)]
    for g in range(2, NG):
        order += _group_names(g) + ['q%d' % g]
    assert sorted(order) == sorted(DMA_NAMES)
    return order


def _pull(gen, n=None):
    if gen is None:
        return
    for _ in (gen if n is None else itertools.islice(gen, n)):
        pass


def _kernel(q_h, k_h, v_h, ssm_h, wg_h, wu_h, wd_h, wm_h,
            sk_ref, dv_ref, c_ref, fm_ref, gm_ref,
            out_h,
            q_v, k_v, v_v, ssm_v, wg_v, wu_v, wd_v, wm_v,
            x_s, k_s, kraw_s, kv_s, y_s, yt_s, x2_s, h2_s, p_s, o_s, vec_s, dn_s, yacc_s, fg_s,
            bar_s, sems, osems):
    cps = {}

    def mk(name, src, dst):
        cps[name] = pltpu.make_async_copy(src, dst, sems.at[DMA_NAMES.index(name)])

    for g in range(NG):
        rows = pl.ds(g * M, M)
        mk('k%d' % g, k_h.at[rows, :], k_v.at[rows, :])
        mk('v%d' % g, v_h.at[rows, :], v_v.at[rows, :])
        mk('q%d' % g, q_h.at[rows, :], q_v.at[rows, :])
    for c in range(NCH):
        mk('s%d' % c, ssm_h.at[:, pl.ds(c * C, C)], ssm_v.at[c])
    for i in range(6 * ND):
        mk('wm%d' % i, wm_h.at[:, pl.ds(i * 128, 128)], wm_v.at[i])
    for f in range(NF):
        mk('wg%d' % f, wg_h.at[:, pl.ds(f * 128, 128)], wg_v.at[f])
        mk('wu%d' % f, wu_h.at[:, pl.ds(f * 128, 128)], wu_v.at[f])
    for j in range(ND):
        mk('wd%d' % j, wd_h.at[:, pl.ds(j * 128, 128)], wd_v.at[j])

    def cp_o(g):
        rows = pl.ds(g * M, M)
        return pltpu.make_async_copy(o_s.at[rows, :], out_h.at[rows, :], osems.at[g])

    def cp_o_last(j):
        rows, cols = pl.ds((NG - 1) * M, M), pl.ds(j * 128, 128)
        return pltpu.make_async_copy(o_s.at[rows, cols], out_h.at[rows, cols], osems.at[NG + j])

    waited = set()

    def W(name):
        if name not in waited:
            waited.add(name)
            cps[name].wait()

    names = _dma_order()
    started = [0]

    def start_more(n):
        for name in names[started[0]:started[0] + n]:
            cps[name].start()
        started[0] = min(started[0] + n, len(names))

    def barrier():
        cpb = pltpu.make_async_copy(bar_s.at[0], bar_s.at[1], osems.at[NG + ND])
        cpb.start()
        cpb.wait()

    start_more(FIRST_DMA_BATCH)

    wg_u, wu_u, wd_u, ssm_u, wm_u = (r.bitcast(u32) for r in (wg_v, wu_v, wd_v, ssm_v, wm_v))
    kv_u, y_u, h2_u, p_u, fg_u = (r.bitcast(u32) for r in (kv_s, y_s, h2_s, p_s, fg_s))

    bar_s[0] = jnp.zeros((8, 128), f32)
    fg_s[0] = fm_ref[...]
    fg_s[1, 0:128] = gm_ref[:, 0:128]
    fg_s[1, 128:256] = gm_ref[:, 128:256]

    def Fm():
        return _unpack(fg_u[0])

    def Gm():
        return jnp.concatenate([_unpack(fg_u[1, 0:64]), _unpack(fg_u[1, 64:128])], axis=1)

    V_W, V_D, V_A1G, V_SAG, V_A2, V_SB, V_GB = 0, 4, 5, 6, 7, 8, 9
    skT = sk_ref[...].astype(f32)
    for j in range(4):
        vec_s[V_W + j] = jnp.broadcast_to(skT[j:j + 1, :], (8, D))
    vec_s[V_D] = jnp.broadcast_to(dv_ref[...].astype(f32).reshape(1, D), (8, D))
    mask8 = jnp.broadcast_to(skT[0:1, 0:128], (8, 128)) * 0.0 > 1.0

    def mask_fn(shape):
        if shape == (8, 128):
            return mask8
        return jnp.concatenate([mask8] * (shape[1] // 128), axis=1)

    def chains_of(n):
        return [Chain(mask_fn) for _ in range(n)]

    def mac_chains(n):
        return [(Chain(mask_fn), Chain(mask_fn)) for _ in range(n)]

    def silu_c():
        cc = c_ref[...].astype(f32)
        return jnp.broadcast_to((cc * jax.nn.sigmoid(cc)).astype(bf16), (16, D))

    def compute_mod():
        s16 = silu_c()
        mods = []
        for i in range(5):
            for j in range(ND):
                W('wm%d' % (i * ND + j))
            mods.append(jnp.concatenate(
                [_dot(s16, _unpack(wm_u[i * ND + j]))[0:8, :] for j in range(ND)], axis=1))
        vec_s[V_A1G] = (1 + mods[1]) * mods[2]
        vec_s[V_SAG] = mods[0] * mods[2]
        vec_s[V_A2] = 1 + mods[4]
        vec_s[V_SB] = mods[3]

    row8 = jax.lax.broadcasted_iota(jnp.int32, (8, 128), 0)
    rowlt = [row8 < j for j in range(3)]

    def KV(c, chains):
        g = c // CPG
        W('k%d' % g)
        W('v%d' % g)
        r0 = c * C

        def wv(j, cs):
            return vec_s[V_W + j, :, cs]

        def shift(prev, cur, j):
            pz = jnp.zeros((8, 128), f32) if prev is None else prev
            return jnp.where(rowlt[j], pltpu.roll(pz, j, 0), pltpu.roll(cur, j, 0))

        prev = [None] * ND
        prevb = [None] * ND
        if c > 0:
            pv = k_v[pl.ds(r0 - 16, 16), :].astype(f32)
            for cc in range(ND):
                cs = slice(cc * 128, (cc + 1) * 128)
                prev[cc] = pv[8:16, cs]
                prevb[cc] = pv[8:16, cs] * wv(2, cs) + shift(pv[0:8, cs], pv[8:16, cs], 1) * wv(3, cs)
        n = 0
        for r in range(r0, r0 + C, 16):
            kvs = []
            k16 = k_v[pl.ds(r, 16), :].astype(f32)
            v16 = v_v[pl.ds(r, 16), :].astype(f32)
            for hh in (0, 8):
                outs = []
                for cc in range(ND):
                    cs = slice(cc * 128, (cc + 1) * 128)
                    ch = chains[n % len(chains)]
                    n += 1
                    kc = ch.link(k16[hh:hh + 8, cs])
                    s1 = shift(prev[cc], kc, 1)
                    a = kc * wv(0, cs) + s1 * wv(1, cs)
                    b = kc * wv(2, cs) + s1 * wv(3, cs)
                    kvc = (a + shift(prevb[cc], b, 2)) * v16[hh:hh + 8, cs]
                    ch.set(kvc)
                    outs.append(kvc)
                    prev[cc] = kc
                    prevb[cc] = b
                kvs.append(outs)
            for j in range(ND):
                kv_s[j, pl.ds(r, 16), :] = jnp.concatenate([kvs[0][j], kvs[1][j]], 0).astype(bf16)
            yield

    def XT(c):
        kvb = jnp.concatenate(
            [_unpack(kv_u[j, pl.ds(c * C // 2, C // 2), :]) for j in range(ND)], axis=1)
        x_s[c] = _dot(Fm(), kvb)

    def KT(c):
        W('s%d' % c)
        kc = _dot_nt(Fm(), _unpack(ssm_u[c]))
        if c == 0:
            k_s[c] = kc
        else:
            kp = kraw_s[(c - 1) % 2]
            k_s[c, 0:64, :] = kc[0:64] - kp[128:192]
            k_s[c, 64:128, :] = kc[64:128] + kp[192:256]
            k_s[c, 128:192, :] = kc[128:192] + kp[0:64]
            k_s[c, 192:256, :] = kc[192:256] - kp[64:128]
        if c < NCH - 1:
            kraw_s[c % 2] = kc

    def MAC(segs, chains):
        npos = 0
        for (i, js, first, last) in segs:
            for r0 in range(0, 128, 16):
                for c0 in range(0, D, 128):
                    res = []
                    for rr in (r0, r0 + 8):
                        chr_, chi_ = chains[npos % len(chains)]
                        npos += 1
                        re, im, cs = slice(rr, rr + 8), slice(128 + rr, 136 + rr), slice(c0, c0 + 128)
                        ar = ai = None
                        if not first:
                            ar = chr_.link(yacc_s[i, re, cs])
                            ai = chi_.link(yacc_s[i, im, cs])
                        for j in js:
                            xr, xi = x_s[j, re, cs], x_s[j, im, cs]
                            kr, ki = k_s[i - j, re, cs], k_s[i - j, im, cs]
                            if ar is None:
                                ar = chr_.link(xr * kr) - xi * ki
                                ai = chi_.link(xr * ki) + xi * kr
                            else:
                                ar = ar + xr * kr
                                ai = ai + xr * ki
                                ar = ar - xi * ki
                                ai = ai + xi * kr
                        chr_.set(ar)
                        chi_.set(ai)
                        res.append((ar, ai))
                        if not last:
                            yacc_s[i, re, cs] = ar
                            yacc_s[i, im, cs] = ai
                    if last:
                        y_s[i, c0 // 128, r0:r0 + 16, :] = (
                            jnp.concatenate([res[0][0], res[1][0]], 0).astype(bf16))
                        y_s[i, c0 // 128, 128 + r0:144 + r0, :] = (
                            jnp.concatenate([res[0][1], res[1][1]], 0).astype(bf16))
                    yield

    def anchored(w, anchors):
        if not anchors:
            return w
        w0 = w[0:8]
        for a in anchors:
            w0 = jnp.where(mask8, pltpu.bitcast(a, u32), w0)
        return jnp.concatenate([w0, w[8:]], axis=0)

    def INV(c, anchors=()):
        yb = jnp.concatenate(
            [_unpack(anchored(y_u[c, j], anchors if j == 0 else ())) for j in range(ND)], axis=1)
        yt_s[c % CPG] = _dot(Gm(), yb)

    def ln(x):
        m = jnp.mean(x, axis=-1, keepdims=True)
        d = x - m
        var = jnp.mean(d * d, axis=-1, keepdims=True)
        return d * jax.lax.rsqrt(var + 1e-5)

    def LN1(g, chains):
        W('q%d' % g)
        n = 0
        for r in range(g * M, (g + 1) * M, 16):
            q16 = q_v[pl.ds(r, 16), :].astype(f32)
            for hh in (0, 8):
                ch = chains[n % len(chains)]
                n += 1
                dn = ln(ch.link(q16[hh:hh + 8]))
                ch.set(dn)
                dn_s[pl.ds(r + hh, 8), :] = dn
            yield

    def POST(g, chains):
        n = 0
        for r in range(g * M, (g + 1) * M, 16):
            c, rl = r // C, r % C
            hs = []
            kvv = jnp.concatenate(
                [_unpack(kv_u[j, pl.ds(r // 2, 8), :]) for j in range(ND)], axis=1).astype(f32)
            q16 = q_v[pl.ds(r, 16), :].astype(f32)
            for hh in (0, 8):
                ch = chains[n % len(chains)]
                n += 1
                y = ch.link(yt_s[c % CPG, rl + hh:rl + hh + 8, :])
                y = y + kvv[hh:hh + 8] * vec_s[V_D]
                hg = dn_s[pl.ds(r + hh, 8), :] * vec_s[V_A1G] + vec_s[V_SAG]
                x2 = q16[hh:hh + 8] + hg * y
                x2_s[pl.ds(r + hh, 8), :] = x2
                h2 = ln(x2) * vec_s[V_A2] + vec_s[V_SB]
                ch.set(h2)
                hs.append(h2)
            hp = jnp.concatenate(hs, 0).astype(bf16)
            for j in range(ND):
                h2_s[j, pl.ds(r, 16), :] = hp[:, j * 128:(j + 1) * 128]
            yield

    def GU(g, f):
        h = jnp.concatenate(
            [_unpack(h2_u[j, pl.ds(g * M // 2, M // 2), :]) for j in range(ND)], axis=1)
        W('wg%d' % f)
        W('wu%d' % f)
        gg = _dot(h, _unpack(wg_u[f]))
        uu = _dot(h, _unpack(wu_u[f]))
        p_s[g % 2, f] = (gg * uu).astype(bf16)

    def DN(g, j):
        p = jnp.concatenate([_unpack(p_u[g % 2, f]) for f in range(NF)], axis=1)
        W('wd%d' % j)
        o = _dot(p, _unpack(wd_u[j]))
        cs = slice(j * 128, (j + 1) * 128)
        gb = jnp.concatenate([vec_s[V_GB][:, cs]] * (M // 8), axis=0)
        o_s[pl.ds(g * M, M), cs] = (x2_s[pl.ds(g * M, M), cs] + gb * o).astype(bf16)
        if g == NG - 1:
            cp_o_last(j).start()
        elif j == ND - 1:
            cp_o(g).start()

    sched = _mac_schedule()
    kvc = chains_of(2)
    pro = [c for g in T_PROLOGUE for c in range(g * CPG, (g + 1) * CPG)]
    for name in _group_names(0):
        W(name)
    _pull(KV(0, kvc))
    for c in pro:
        if c + 1 in pro:
            if (c + 1) % CPG == 0:
                for name in _group_names((c + 1) // CPG):
                    W(name)
            _pull(KV(c + 1, kvc))
        XT(c)
        KT(c)
    extra, due = sched[0]
    mc0 = mac_chains(2)
    _pull(MAC(due, mc0))
    for c in range(CPG):
        INV(c)
    W('q0')
    W('q1')
    ln_chains = chains_of(8)
    _pull(LN1(0, ln_chains))
    _pull(LN1(1, ln_chains))
    _pull(MAC(extra, mc0))
    start_more(SECOND_DMA_BATCH)
    compute_mod()
    _pull(POST(0, chains_of(16)))

    for s in range(1, NG + 1):
        g = s - 1
        tg = T_PLACE.get(s)
        if s == 2:
            start_more(len(names))
        if 2 <= s < NG:
            W('q%d' % s)
            if tg is not None:
                W('k%d' % tg)
                W('v%d' % tg)

        mac, nm = None, 0
        if s < NG:
            extra, due = sched[s]
            if s > 1:
                _pull(LN1(s, chains_of(3)))
            mch = mac_chains(1)
            mac = MAC(extra + due, mch)
            nm = len(extra + due) * 40
        for f in range(NF):
            if s == 1:
                for ff in GU_WAITS.get(f, ()):
                    W('wg%d' % ff)
                    W('wu%d' % ff)
            GU(g, f)
            if s == 1:
                _pull(mac, (nm * (f + 1)) // NF - (nm * f) // NF)
        _pull(mac)

        post = None
        if s < NG:
            INV(s * CPG, (mch[0][0].prev, mch[0][1].prev) if nm > 0 else ())
            INV(s * CPG + 1)
            post = POST(s, chains_of(3))
        for j in range(ND):
            if s == 1:
                W('wd%d' % j)
                W('wm%d' % (5 * ND + j))
                vec_s[V_GB, :, j * 128:(j + 1) * 128] = (
                    _dot(silu_c(), _unpack(wm_u[5 * ND + j]))[0:8, :])
            DN(g, j)
            if s == 1:
                _pull(post, ((M // 16) * (j + 1)) // ND - ((M // 16) * j) // ND)
        _pull(post)

        if tg is not None:
            c0 = tg * CPG
            if s > 1:
                kc = chains_of(3)
                for c in range(c0, c0 + CPG):
                    _pull(KV(c, kc))
            barrier()
            for name in _group_names(tg):
                W(name)
            if s == 1:
                kc = chains_of(2)
                for c in range(c0, c0 + CPG):
                    _pull(KV(c, kc))
            for c in range(c0, c0 + CPG):
                XT(c)
                KT(c)
            barrier()

    for name in names:
        W(name)
    for g in range(NG - 1):
        cp_o(g).wait()
    for j in range(ND):
        cp_o_last(j).wait()


@jax.jit
def pallas_adaLN_cond__ssm_conv_h3__glu_gated_bilinear__prompt_kernel(
    A_q: jax.Array,
    A_k: jax.Array,
    A_v: jax.Array,
    A_shift_k: jax.Array,
    A_ssm_k: jax.Array,
    A_ssm_D: jax.Array,
    B_x: jax.Array,
    B_w_gate: jax.Array,
    B_w_up: jax.Array,
    B_w_down: jax.Array,
    c: jax.Array,
    w_mod: jax.Array,
):
    del B_x
    fm, gm = _dft_consts()
    fm = jnp.asarray(fm, dtype=bf16)
    gm = jnp.asarray(gm, dtype=bf16)
    any_spec = pl.BlockSpec(memory_space=pl.ANY)
    vmem_spec = pl.BlockSpec(memory_space=pltpu.VMEM)
    out = pl.pallas_call(
        _kernel,
        in_specs=[any_spec] * 8 + [vmem_spec] * 5,
        out_specs=any_spec,
        out_shape=jax.ShapeDtypeStruct((S, D), bf16),
        scratch_shapes=[
            pltpu.VMEM((S, D), bf16), pltpu.VMEM((S, D), bf16), pltpu.VMEM((S, D), bf16),
            pltpu.VMEM((NCH, D, C), bf16),
            pltpu.VMEM((NF, D, 128), bf16), pltpu.VMEM((NF, D, 128), bf16),
            pltpu.VMEM((ND, F, 128), bf16),
            pltpu.VMEM((6 * ND, D, 128), bf16),
            pltpu.VMEM((NCH, 256, D), f32), pltpu.VMEM((NCH, 256, D), f32),
            pltpu.VMEM((2, 256, D), f32),
            pltpu.VMEM((ND, S, 128), bf16),
            pltpu.VMEM((NCH, ND, 256, 128), bf16), pltpu.VMEM((CPG, C, D), f32),
            pltpu.VMEM((S, D), f32), pltpu.VMEM((ND, S, 128), bf16),
            pltpu.VMEM((2, NF, M, 128), bf16), pltpu.VMEM((S, D), bf16),
            pltpu.VMEM((10, 8, D), f32), pltpu.VMEM((S, D), f32),
            pltpu.VMEM((NCH, 256, D), f32),
            pltpu.VMEM((2, 256, 128), bf16), pltpu.VMEM((2, 8, 128), f32),
            pltpu.SemaphoreType.DMA((len(DMA_NAMES),)),
            pltpu.SemaphoreType.DMA((NG + ND + 1,)),
        ],
        compiler_params=pltpu.CompilerParams(vmem_limit_bytes=110 * 1024 * 1024),
    )(A_q.reshape(S, D), A_k.reshape(S, D), A_v.reshape(S, D), A_ssm_k, B_w_gate, B_w_up, B_w_down,
      w_mod, A_shift_k.T, A_ssm_D, c, fm, gm)
    return out.reshape(1, S, D)
```
